```python
import os as _os
_os.environ.setdefault('JAX_PLATFORMS', 'cpu')
import jax
import jax.numpy as jnp

def _softmax(x, axis=-1):
    return jax.nn.softmax(x, axis=axis)

def _gelu(x):
    return jax.nn.gelu(x, approximate=True)

def _silu(x):
    return jax.nn.silu(x)

def _sigmoid(x):
    return jax.nn.sigmoid(x)

def _layernorm(x, axis=-1, eps=1e-05):
    m = jnp.mean(x, axis=axis, keepdims=True)
    v = jnp.var(x, axis=axis, keepdims=True)
    return (x - m) / jnp.sqrt(v + eps)

def _scatter_add(tgt, idx, src, axis=0):
    return tgt.at[idx].add(src)

def _segment_sum(src, seg, n):
    return jax.ops.segment_sum(src, seg, n)

class _Rng:

    def __init__(self, key):
        self._k = key

    def _next(self):
        self._k, sub = jax.random.split(self._k)
        return sub

    def normal(self, shape):
        return jax.random.normal(self._next(), shape, dtype=jnp.bfloat16)

    def randint(self, lo, hi, shape):
        return jax.random.randint(self._next(), shape, lo, hi, dtype=jnp.int32)

    def uniform(self, shape, lo=0.0, hi=1.0):
        return jax.random.uniform(self._next(), shape, jnp.bfloat16, lo, hi)

    def permutation(self, n):
        return jax.random.permutation(self._next(), n)
kernel_name = 'standalone__autoregressive_conv_wavenet__speech'

def setup_inputs():
    _rng = _Rng(jax.random.key(int.from_bytes(__import__("os").urandom(4), "little")))
    _w = lambda a: (lambda t: t.astype(jnp.bfloat16) if jnp.issubdtype(t.dtype, jnp.floating) else t)(jnp.asarray(a))
    B, T, D, K = (2, 4000, 512, 31)
    return {'x': _w((lambda *s: _rng.normal(s) * 0.05)(B, T, D)), 'w': _w((lambda *s: _rng.normal(s) * 0.05)(K, D, 2 * D)), 'w_o': _w((lambda *s: _rng.normal(s) * 0.05)(D, D))}

def reference(x, w, w_o):
    B, T, D = x.shape
    K = w.shape[0]
    dil = 2
    pad = (K - 1) * dil
    xp = jnp.pad(x, ((0, 0), (pad, 0), (0, 0)))
    h = jnp.einsum('btc,cd->btd', xp[:, pad:pad + T, :], w[0])
    for i in range(1, K):
        off = pad - i * dil
        h = h + jnp.einsum('btc,cd->btd', xp[:, off:off + T, :], w[i])
    f = h[..., :D].copy()
    g = h[..., D:].copy()
    z = jnp.tanh(f) * _sigmoid(g)
    return z @ w_o
```

```python
import functools
import jax
import jax.numpy as jnp
import jax.experimental.pallas as pl
import jax.experimental.pallas.tpu as pltpu

DIL = 2
ROW_TILE = 16
G = ROW_TILE // DIL
HALO = 64


def _kernel(x_ref, w_hbm, wo_ref, o_ref, xs_ref, acc_ref, w_vmem, w_sems, *, K, T, D, BN, EC):
    b = pl.program_id(0)
    NB = (2 * D) // BN
    n_grp = -(-K // G)
    last_j = K - (n_grp - 1) * G

    def slice_copy(a, nb):
        s0 = jnp.minimum(G * a, K - G)
        col = pl.multiple_of(nb * BN, BN)
        return pltpu.make_async_copy(
            w_hbm.at[pl.ds(s0, G), :, pl.ds(col, BN)],
            w_vmem.at[pl.ds(G * a, G), :, pl.ds(col, BN)],
            w_sems.at[a * NB + nb])

    @pl.when(b == 0)
    def _():
        for a in range(n_grp):
            for nb in range(NB):
                slice_copy(a, nb).start()

    xs_ref[0:HALO, :] = jnp.zeros((HALO, D), xs_ref.dtype)
    xs_ref[HALO:HALO + T, :] = x_ref[0]

    def tap_dot(a, j, col):
        base = pl.multiple_of(HALO - ROW_TILE - ROW_TILE * a, ROW_TILE)
        xw = xs_ref[pl.ds(base, T + ROW_TILE), :]
        xi = xw[ROW_TILE - DIL * j:ROW_TILE - DIL * j + T, :]
        slot = G * a + j + jnp.where(a == n_grp - 1, G - last_j, 0)
        wi = w_vmem[slot, :, pl.ds(col, BN)]
        c = jnp.dot(xi, wi, preferred_element_type=jnp.float32)
        if j == 0:
            acc_ref[:, pl.ds(col, BN)] = jnp.where(a == 0, c, acc_ref[:, pl.ds(col, BN)] + c)
        else:
            acc_ref[:, pl.ds(col, BN)] += c

    def taps_over_cols(a, js, wait_slice):
        def nb_body(nb, carry):
            col = pl.multiple_of(nb * BN, BN)
            if wait_slice:
                slice_copy(a, nb).wait()
            for j in js:
                tap_dot(a, j, col)
            return carry
        jax.lax.fori_loop(0, NB, nb_body, 0)

    def a_body(a, carry):
        taps_over_cols(a, range(last_j), wait_slice=True)

        @pl.when(a < n_grp - 1)
        def _():
            taps_over_cols(a, range(last_j, G), wait_slice=False)

        for nb in range(NB):
            slice_copy(a, nb).start()
        return carry

    jax.lax.fori_loop(0, n_grp, a_body, 0)

    def ep_body(c, carry):
        r0 = pl.multiple_of(c * EC, ROW_TILE)
        f = acc_ref[pl.ds(r0, EC), 0:D]
        g = acc_ref[pl.ds(r0, EC), D:2 * D]
        z = jnp.tanh(f) * (0.5 * jnp.tanh(0.5 * g) + 0.5)
        o_ref[0, pl.ds(r0, EC), :] = jnp.dot(
            z.astype(jnp.bfloat16), wo_ref[...],
            preferred_element_type=jnp.float32).astype(o_ref.dtype)
        return carry

    jax.lax.fori_loop(0, T // EC, ep_body, 0)

    @pl.when(b == pl.num_programs(0) - 1)
    def _():
        for a in range(n_grp):
            for nb in range(NB):
                slice_copy(a, nb).wait()


@jax.jit
def pallas_standalone__autoregressive_conv_wavenet__speech_kernel(x, w, w_o):
    B, T, D = x.shape
    K = w.shape[0]
    BN = 256
    EC = 800
    assert T % EC == 0 and EC % ROW_TILE == 0 and (2 * D) % BN == 0 and BN % 128 == 0
    assert HALO >= (K - 1) * DIL and T % ROW_TILE == 0
    kernel = functools.partial(_kernel, K=K, T=T, D=D, BN=BN, EC=EC)
    return pl.pallas_call(
        kernel,
        grid=(B,),
        in_specs=[
            pl.BlockSpec((1, T, D), lambda b: (b, 0, 0)),
            pl.BlockSpec(memory_space=pl.ANY),
            pl.BlockSpec((D, D), lambda b: (0, 0)),
        ],
        out_specs=pl.BlockSpec((1, T, D), lambda b: (b, 0, 0)),
        out_shape=jax.ShapeDtypeStruct((B, T, D), x.dtype),
        scratch_shapes=[
            pltpu.VMEM((HALO + T, D), jnp.bfloat16),
            pltpu.VMEM((T, 2 * D), jnp.float32),
            pltpu.VMEM((-(-K // G) * G, D, 2 * D), jnp.bfloat16),
            pltpu.SemaphoreType.DMA((-(-K // G) * ((2 * D) // BN),)),
        ],
        compiler_params=pltpu.CompilerParams(
            dimension_semantics=("arbitrary",),
            vmem_limit_bytes=110 * 1024 * 1024,
        ),
    )(x, w, w_o)
```
